```python
import os as _os
_os.environ.setdefault("JAX_PLATFORMS", "cpu")
import jax
import jax.numpy as jnp

def _softmax(x, axis=-1):
    return jax.nn.softmax(x, axis=axis)
def _gelu(x):
    return jax.nn.gelu(x, approximate=True)
def _silu(x):
    return jax.nn.silu(x)
def _sigmoid(x):
    return jax.nn.sigmoid(x)
def _layernorm(x, axis=-1, eps=1e-5):
    m = jnp.mean(x, axis=axis, keepdims=True)
    v = jnp.var(x, axis=axis, keepdims=True)
    return (x - m) / jnp.sqrt(v + eps)
def _scatter_add(tgt, idx, src, axis=0):
    return tgt.at[idx].add(src)
def _segment_sum(src, seg, n):
    return jax.ops.segment_sum(src, seg, n)
class _Rng:
    def __init__(self, key):
        self._k = key
    def _next(self):
        self._k, sub = jax.random.split(self._k)
        return sub
    def normal(self, shape):
        return jax.random.normal(self._next(), shape, dtype=jnp.bfloat16)
    def randint(self, lo, hi, shape):
        return jax.random.randint(self._next(), shape, lo, hi, dtype=jnp.int32)
    def uniform(self, shape, lo=0.0, hi=1.0):
        return jax.random.uniform(self._next(), shape, jnp.bfloat16, lo, hi)
    def permutation(self, n):
        return jax.random.permutation(self._next(), n)


kernel_name = 'standalone__cross_network_dcn_v2__recsys'

def setup_inputs():
    _rng = _Rng(jax.random.key(int.from_bytes(__import__("os").urandom(4), "little")))
    _w = (lambda a: (lambda t: t.astype(jnp.bfloat16) if jnp.issubdtype(t.dtype, jnp.floating) else t)(jnp.asarray(a)))
    B, F, D, L = 16384, 26, 16, 6
    Din = min(F * D, 512)
    R = max(Din // 4, 2)
    sc = Din ** -0.5
    return {
        "x0": _w((lambda *s: _rng.normal(s) * 0.05)(B, Din)),
        "U":  _w((lambda *s: _rng.normal(s) * 1.6)(L, Din, R) * sc),
        "V":  _w((lambda *s: _rng.normal(s) * 1.6)(L, R, Din) * sc),
        "bs": _w((lambda *s: _rng.normal(s) * 0.05)(L, Din)),
    }

def reference(x0, U, V, bs):
    x = x0
    for l in range(U.shape[0]):
        h = jnp.einsum('rd,bd->br', V[l], x)
        h = jnp.einsum('dr,br->bd', U[l], h)
        x = x0 * (h + bs[l]) + x
    return x
```

```python
import functools

import jax
import jax.numpy as jnp
import jax.experimental.pallas as pl
import jax.experimental.pallas.tpu as pltpu


def _kernel(x0_ref, u_ref, v_ref, b_ref, o_ref, *, n_layers):
    x0b = x0_ref[...]
    x0 = x0b.astype(jnp.float32)
    x = x0b
    s = None
    for l in range(n_layers):
        h = jnp.dot(v_ref[l], x, preferred_element_type=jnp.float32)
        y = jnp.dot(u_ref[l], h.astype(jnp.bfloat16), preferred_element_type=jnp.float32)
        y = y + b_ref[l].astype(jnp.float32)
        s = (y + 1.0) if s is None else (s + y)
        x = (x0 * s).astype(jnp.bfloat16)
    o_ref[...] = x


@jax.jit
def pallas_standalone__cross_network_dcn_v2__recsys_kernel(x0, U, V, bs):
    B, D = x0.shape
    L, _, R = U.shape
    TB = 512
    x0t = x0.T
    bcol = bs.reshape(L, D, 1)
    out_t = pl.pallas_call(
        functools.partial(_kernel, n_layers=L),
        grid=(B // TB,),
        in_specs=[
            pl.BlockSpec((D, TB), lambda i: (0, i)),
            pl.BlockSpec((L, D, R), lambda i: (0, 0, 0)),
            pl.BlockSpec((L, R, D), lambda i: (0, 0, 0)),
            pl.BlockSpec((L, D, 1), lambda i: (0, 0, 0)),
        ],
        out_specs=pl.BlockSpec((D, TB), lambda i: (0, i)),
        out_shape=jax.ShapeDtypeStruct((D, B), x0.dtype),
        compiler_params=pltpu.CompilerParams(
            dimension_semantics=("parallel",),
            vmem_limit_bytes=64 * 1024 * 1024,
        ),
    )(x0t, U, V, bcol)
    return out_t.T
```

```python
import functools

import jax
import jax.numpy as jnp
from jax import lax
import jax.experimental.pallas as pl
import jax.experimental.pallas.tpu as pltpu

F32 = jnp.float32
BF16 = jnp.bfloat16
U32 = jnp.uint32

W = 128
KA = 384
NC = 9
RP = 112


def _pk(x):
    return pltpu.bitcast(x, U32)


def _upk(x):
    return pltpu.bitcast(x, BF16)


def _kernel(x0_hbm, u_hbm, v_hbm, b_hbm, o_hbm,
            u_ref, v_ref, b_ref, bt_ref, uw_ref, va_ref, vcb_ref,
            x0f_ref, s_ref, xa_ref, xr_ref, st_ref,
            xin0_ref, xout0_ref, xin_ref, xout_ref, w_sem, in_sem, out_sem, *,
            G0, d0, G, d, U, OG, L0, lead, nfine):
    D, B = x0_hbm.shape
    L, _, R = u_ref.shape
    C0 = G0 * W
    CI = U * G * W
    NI = (B - C0) // CI
    assert NI * CI + C0 == B and NI >= 2
    half = [(0, 208), (208, D)]
    fine = [(0, 112), (112, 208), (208, 320), (320, D)]

    def cols(i, off, n):
        return pl.ds(pl.multiple_of(C0 + i * CI + off, W), n)

    def in_copy(i, par):
        return pltpu.make_async_copy(
            x0_hbm.at[:, cols(i, 0, CI)], xin_ref.at[par], in_sem.at[par])

    def out_copy(i, par, c0, n):
        return pltpu.make_async_copy(
            xout_ref.at[par, :, pl.ds(c0, n)], o_hbm.at[:, cols(i, c0, n)],
            out_sem.at[par])

    def out_wait_all(par):
        pltpu.make_async_copy(
            xout_ref.at[par], xout_ref.at[par], out_sem.at[par]).wait()

    first = [
        pltpu.make_async_copy(v_hbm.at[0:L0], v_ref.at[0:L0], w_sem.at[0]),
        pltpu.make_async_copy(b_hbm, b_ref, w_sem.at[1]),
        pltpu.make_async_copy(u_hbm.at[0:L0], u_ref.at[0:L0], w_sem.at[2]),
        pltpu.make_async_copy(x0_hbm.at[:, 0:C0], xin0_ref, w_sem.at[3]),
    ]
    second = [
        pltpu.make_async_copy(v_hbm.at[L0:L], v_ref.at[L0:L], w_sem.at[4]),
        pltpu.make_async_copy(u_hbm.at[L0:L], u_ref.at[L0:L], w_sem.at[5]),
    ]
    out0 = pltpu.make_async_copy(xout0_ref, o_hbm.at[:, 0:C0], w_sem.at[6])
    for c in first + second:
        c.start()
    in_copy(0, 0).start()
    for c in first[:3]:
        c.wait()

    def vpu_col(l, j):
        return j if j < 8 else 8 + l

    def init_bias():
        b = b_ref[...].astype(F32)
        bm = jnp.concatenate(
            [jnp.zeros((R, D), F32), b, jnp.zeros((128 - R - L, D), F32)], axis=0)
        bm = jnp.concatenate([bm, jnp.zeros((128, 512 - D), F32)], axis=1)
        bt_ref[...] = bm.T[:D]

    def init(l):
        row = lax.broadcasted_iota(jnp.int32, (R, 128), 0)
        col = lax.broadcasted_iota(jnp.int32, (R, 128), 1)
        for k in range(3):
            vk = v_ref[l, :, k * 128:(k + 1) * 128].astype(F32)
            vk = jnp.concatenate([vk, jnp.zeros((RP - R, 128), F32)], axis=0)
            va_ref[l, k] = _pk(vk.astype(BF16))
        vt0 = v_ref[l, :, KA:D].astype(F32)
        for j in range(NC):
            c = vpu_col(l, j)
            vcb_ref[l, j] = jnp.broadcast_to(vt0[:, c:c + 1], (R, 128))
        vt = jnp.concatenate([jnp.zeros((R, 128 - (D - KA)), F32), vt0], axis=1)
        e = jnp.where(col >= R, vt, jnp.where(row == col, 1.0, 0.0)).astype(BF16)
        for (r0, r1) in half:
            cold = lax.broadcasted_iota(jnp.int32, (r1 - r0, 128), 1)
            uw = jnp.dot(u_ref[l, r0:r1, :], e, preferred_element_type=F32)
            uw = jnp.where(cold == R + l, bt_ref[r0:r1, :], uw)
            uw_ref[l, r0 // 2:r1 // 2, :] = _pk(uw.astype(BF16))

    def p1(xin, c0, g, l):
        sub = lax.broadcasted_iota(jnp.int32, (128 - R, W), 0)
        if l == 0:
            x0f_ref[g] = xin[:, c0:c0 + W].astype(F32)
        h = None
        for k in range(3):
            if l == 0:
                xa = xin[k * 128:(k + 1) * 128, c0:c0 + W]
            else:
                xa = xa_ref[g, k * 128:(k + 1) * 128, :]
            p = jnp.dot(_upk(va_ref[l, k]), xa, preferred_element_type=F32)[:R]
            h = p if h is None else h + p
        xr = x0f_ref[g, KA:, :] if l == 0 else xr_ref[g]
        for j in range(NC):
            c = vpu_col(l, j)
            h = h + vcb_ref[l, j] * xr[c:c + 1, :]
        tail = jnp.where(sub == l, 1.0, xr[8:])
        st_ref[g] = jnp.concatenate([h, tail], axis=0).astype(BF16)

    def p2(xout, c0, g, l, chunks):
        st = st_ref[g]
        for (r0, r1) in chunks:
            y = jnp.dot(_upk(uw_ref[l, r0 // 2:r1 // 2, :]), st,
                        preferred_element_type=F32)
            s = (y + 1.0) if l == 0 else (s_ref[g, r0:r1, :] + y)
            x = x0f_ref[g, r0:r1, :] * s
            if l == L - 1:
                xout[r0:r1, c0:c0 + W] = x.astype(BF16)
            else:
                s_ref[g, r0:r1, :] = s
                if r1 <= KA:
                    xa_ref[g, r0:r1, :] = x.astype(BF16)
                else:
                    xa_ref[g, r0:KA, :] = x[:KA - r0].astype(BF16)
                    xr_ref[g] = x[KA - r0:]

    init_bias()
    for l in range(L0):
        init(l)
    first[3].wait()
    ts0 = L * G0
    tb = L0 * G0 - lead
    for t in range(ts0 + d0):
        if (t + lead) % G0 == 0 and L0 <= (t + lead) // G0 < L:
            ln = (t + lead) // G0
            if ln == L0:
                for c in second:
                    c.wait()
            init(ln)
        if t < ts0:
            l, g = divmod(t, G0)
            p1(xin0_ref, g * W, g, l)
        if t >= d0:
            l, g = divmod(t - d0, G0)
            last = t >= ts0 + d0 - nfine or tb - nfine <= t < tb
            p2(xout0_ref, g * W, g, l, fine if last else half)
    out0.start()

    ts = L * G
    nt = ts * U

    def body(i, carry):
        par = lax.rem(i, 2)

        @pl.when(i + 1 < NI)
        def _():
            in_copy(i + 1, 1 - par).start()

        in_copy(i, par).wait()

        @pl.when(i >= 2)
        def _():
            out_wait_all(par)

        xin = xin_ref.at[par]
        xout = xout_ref.at[par]
        done = 0
        for t in range(nt + d):
            if t < nt:
                u, r = divmod(t, ts)
                l, g = divmod(r, G)
                p1(xin, (u * G + g) * W, g, l)
            if t >= d:
                u, r = divmod(t - d, ts)
                l, g = divmod(r, G)
                p2(xout, (u * G + g) * W, g, l,
                   fine if t >= nt + d - nfine else half)
                if l == L - 1:
                    end = (u * G + g + 1) * W
                    rem = G - 1 - g
                    if (rem == 0) if u < U - 1 else (rem in OG):
                        @pl.when(i == NI - 1)
                        def _(done=done, end=end):
                            out_copy(i, par, done, end - done).start()
                        done = end
        assert done == CI

        @pl.when(i < NI - 1)
        def _():
            out_copy(i, par, 0, CI).start()

        return carry

    lax.fori_loop(0, NI, body, 0)
    out0.wait()
    out_wait_all((NI - 2) % 2)
    out_wait_all((NI - 1) % 2)


@jax.jit
def pallas_standalone__cross_network_dcn_v2__recsys_kernel(x0, U, V, bs):
    B, D = x0.shape
    L, _, R = U.shape
    assert (D, R) == (416, 104) and L <= 8
    G0, d0, G, d, NU = 8, 3, 10, 4, 3
    GM = max(G, G0)
    out_t = pl.pallas_call(
        functools.partial(_kernel, G0=G0, d0=d0, G=G, d=d, U=NU, OG=(0, 2, 5),
                          L0=2, lead=4, nfine=3),
        in_specs=[pl.BlockSpec(memory_space=pl.ANY)] * 4,
        out_specs=pl.BlockSpec(memory_space=pl.ANY),
        out_shape=jax.ShapeDtypeStruct((D, B), x0.dtype),
        scratch_shapes=[
            pltpu.VMEM((L, D, R), BF16),
            pltpu.VMEM((L, R, D), BF16),
            pltpu.VMEM((L, D), BF16),
            pltpu.VMEM((D, 128), F32),
            pltpu.VMEM((L, D // 2, 128), U32),
            pltpu.VMEM((L, 3, RP // 2, 128), U32),
            pltpu.VMEM((L, NC, R, 128), F32),
            pltpu.VMEM((GM, D, W), F32),
            pltpu.VMEM((GM, D, W), F32),
            pltpu.VMEM((GM, KA, W), BF16),
            pltpu.VMEM((GM, D - KA, W), F32),
            pltpu.VMEM((GM, 128, W), BF16),
            pltpu.VMEM((D, G0 * W), BF16),
            pltpu.VMEM((D, G0 * W), BF16),
            pltpu.VMEM((2, D, NU * G * W), BF16),
            pltpu.VMEM((2, D, NU * G * W), BF16),
            pltpu.SemaphoreType.DMA((7,)),
            pltpu.SemaphoreType.DMA((2,)),
            pltpu.SemaphoreType.DMA((2,)),
        ],
        compiler_params=pltpu.CompilerParams(
            vmem_limit_bytes=100 * 1024 * 1024,
            disable_bounds_checks=True,
        ),
    )(x0.T, U, V, bs)
    return out_t.T
```

```python
import functools

import jax
import jax.numpy as jnp
from jax import lax
import jax.experimental.pallas as pl
import jax.experimental.pallas.tpu as pltpu

F32 = jnp.float32
BF16 = jnp.bfloat16
U32 = jnp.uint32

W = 128
KA = 384
NC = 9
RP = 112


def _pk(x):
    return pltpu.bitcast(x, U32)


def _upk(x):
    return pltpu.bitcast(x, BF16)


def _kernel(x0_hbm, u_hbm, v_hbm, b_hbm, o_hbm,
            u_ref, v_ref, b_ref, bt_ref, uw_ref, va_ref, vcb_ref,
            x0f_ref, s_ref, xa_ref, xr_ref, st_ref,
            xin0_ref, xout0_ref, xin_ref, xout_ref, w_sem, in_sem, out_sem, *,
            GA, G0, d0, G, d, NU, L0, lead, nfine):
    D, B = x0_hbm.shape
    L, _, R = u_ref.shape
    CA = GA * W
    C0 = G0 * W
    CI = NU * G * W
    NI = (B - C0) // CI
    assert NI * CI + C0 == B and NI >= 2
    half = [(0, 208), (208, D)]
    fine = [(0, 112), (112, 208), (208, 320), (320, D)]

    def cols(i, off, n):
        return pl.ds(pl.multiple_of(C0 + i * CI + off, W), n)

    def in_copy(i, par):
        return pltpu.make_async_copy(
            x0_hbm.at[:, cols(i, 0, CI)], xin_ref.at[par], in_sem.at[par])

    def out_copy(i, par, c0, n):
        return pltpu.make_async_copy(
            xout_ref.at[par, :, pl.ds(c0, n)], o_hbm.at[:, cols(i, c0, n)],
            out_sem.at[par])

    def out_wait_all(par):
        pltpu.make_async_copy(
            xout_ref.at[par], xout_ref.at[par], out_sem.at[par]).wait()

    stage1 = [
        pltpu.make_async_copy(v_hbm.at[0:1], v_ref.at[0:1], w_sem.at[0]),
        pltpu.make_async_copy(b_hbm, b_ref, w_sem.at[1]),
        pltpu.make_async_copy(u_hbm.at[0:1], u_ref.at[0:1], w_sem.at[2]),
        pltpu.make_async_copy(
            x0_hbm.at[:, 0:CA], xin0_ref.at[:, 0:CA], w_sem.at[3]),
    ]
    stage2 = [
        pltpu.make_async_copy(
            x0_hbm.at[:, CA:C0], xin0_ref.at[:, CA:C0], w_sem.at[4]),
        pltpu.make_async_copy(v_hbm.at[1:L0], v_ref.at[1:L0], w_sem.at[5]),
        pltpu.make_async_copy(u_hbm.at[1:L0], u_ref.at[1:L0], w_sem.at[6]),
    ]
    stage3 = [
        pltpu.make_async_copy(v_hbm.at[L0:L], v_ref.at[L0:L], w_sem.at[7]),
        pltpu.make_async_copy(u_hbm.at[L0:L], u_ref.at[L0:L], w_sem.at[8]),
    ]
    out0 = pltpu.make_async_copy(xout0_ref, o_hbm.at[:, 0:C0], w_sem.at[9])
    for c in stage1 + stage2 + stage3:
        c.start()
    in_copy(0, 0).start()

    def vpu_col(l, j):
        return j if j < 8 else 8 + l

    def init_bias():
        b = b_ref[...].astype(F32)
        bm = jnp.concatenate(
            [jnp.zeros((R, D), F32), b, jnp.zeros((128 - R - L, D), F32)], axis=0)
        bm = jnp.concatenate([bm, jnp.zeros((128, 512 - D), F32)], axis=1)
        bt_ref[...] = bm.T[:D]

    def init(l):
        row = lax.broadcasted_iota(jnp.int32, (R, 128), 0)
        col = lax.broadcasted_iota(jnp.int32, (R, 128), 1)
        for k in range(3):
            vk = v_ref[l, :, k * 128:(k + 1) * 128].astype(F32)
            vk = jnp.concatenate([vk, jnp.zeros((RP - R, 128), F32)], axis=0)
            va_ref[l, k] = _pk(vk.astype(BF16))
        vt0 = v_ref[l, :, KA:D].astype(F32)
        for j in range(NC):
            c = vpu_col(l, j)
            vcb_ref[l, j] = jnp.broadcast_to(vt0[:, c:c + 1], (R, 128))
        vt = jnp.concatenate([jnp.zeros((R, 128 - (D - KA)), F32), vt0], axis=1)
        e = jnp.where(col >= R, vt, jnp.where(row == col, 1.0, 0.0)).astype(BF16)
        for r0 in range(0, D, 112):
            r1 = min(r0 + 112, D)
            cold = lax.broadcasted_iota(jnp.int32, (r1 - r0, 128), 1)
            uw = jnp.dot(u_ref[l, r0:r1, :], e, preferred_element_type=F32)
            uw = jnp.where(cold == R + l, bt_ref[r0:r1, :], uw)
            uw_ref[l, r0 // 2:r1 // 2, :] = _pk(uw.astype(BF16))

    def p1(xin, c0, g, l):
        sub = lax.broadcasted_iota(jnp.int32, (128 - R, W), 0)
        if l == 0:
            x0f_ref[g] = xin[:, c0:c0 + W].astype(F32)
        h = None
        for k in range(3):
            if l == 0:
                xa = xin[k * 128:(k + 1) * 128, c0:c0 + W]
            else:
                xa = xa_ref[g, k * 128:(k + 1) * 128, :]
            p = jnp.dot(_upk(va_ref[l, k]), xa, preferred_element_type=F32)[:R]
            h = p if h is None else h + p
        xr = x0f_ref[g, KA:, :] if l == 0 else xr_ref[g]
        for j in range(NC):
            c = vpu_col(l, j)
            h = h + vcb_ref[l, j] * xr[c:c + 1, :]
        tail = jnp.where(sub == l, 1.0, xr[8:])
        st_ref[g] = jnp.concatenate([h, tail], axis=0).astype(BF16)

    def p2(xout, c0, g, l, chunks):
        st = st_ref[g]
        for (r0, r1) in chunks:
            y = jnp.dot(_upk(uw_ref[l, r0 // 2:r1 // 2, :]), st,
                        preferred_element_type=F32)
            s = (y + 1.0) if l == 0 else (s_ref[g, r0:r1, :] + y)
            x = x0f_ref[g, r0:r1, :] * s
            if l == L - 1:
                xout[r0:r1, c0:c0 + W] = x.astype(BF16)
            else:
                s_ref[g, r0:r1, :] = s
                if r1 <= KA:
                    xa_ref[g, r0:r1, :] = x.astype(BF16)
                else:
                    xa_ref[g, r0:KA, :] = x[:KA - r0].astype(BF16)
                    xr_ref[g] = x[KA - r0:]

    for c in stage1[:3]:
        c.wait()
    init_bias()
    init(0)
    stage1[3].wait()
    for g in range(GA):
        p1(xin0_ref, g * W, g, 0)
    for g in range(GA):
        p2(xout0_ref, g * W, g, 0, fine)
    for c in stage2:
        c.wait()
    for l in range(1, L0):
        init(l)
    ts0 = L * G0
    tb = L0 * G0 - lead
    for t in range(GA, ts0 + d0):
        if (t + lead) % G0 == 0 and L0 <= (t + lead) // G0 < L:
            ln = (t + lead) // G0
            if ln == L0:
                for c in stage3:
                    c.wait()
            init(ln)
        if t < ts0:
            l, g = divmod(t, G0)
            p1(xin0_ref, g * W, g, l)
        if t - d0 >= GA:
            l, g = divmod(t - d0, G0)
            last = t >= ts0 + d0 - nfine or tb - nfine <= t < tb
            p2(xout0_ref, g * W, g, l, fine if last else half)
    out0.start()

    ts = L * G
    nt = ts * NU

    def body(i, carry):
        par = lax.rem(i, 2)

        @pl.when(i + 1 < NI)
        def _():
            in_copy(i + 1, 1 - par).start()

        in_copy(i, par).wait()

        @pl.when(i >= 2)
        def _():
            out_wait_all(par)

        xin = xin_ref.at[par]
        xout = xout_ref.at[par]
        done = 0
        for t in range(nt + d):
            if t < nt:
                u, r = divmod(t, ts)
                l, g = divmod(r, G)
                p1(xin, (u * G + g) * W, g, l)
            if t >= d:
                u, r = divmod(t - d, ts)
                l, g = divmod(r, G)
                p2(xout, (u * G + g) * W, g, l,
                   fine if t >= nt + d - nfine else half)
                if l == L - 1 and (u == NU - 1 or g == G - 1):
                    end = (u * G + g + 1) * W

                    @pl.when(i == NI - 1)
                    def _(done=done, end=end):
                        out_copy(i, par, done, end - done).start()

                    done = end
        assert done == CI

        @pl.when(i < NI - 1)
        def _():
            out_copy(i, par, 0, CI).start()

        return carry

    lax.fori_loop(0, NI, body, 0)
    out0.wait()
    out_wait_all((NI - 2) % 2)
    out_wait_all((NI - 1) % 2)


@jax.jit
def pallas_standalone__cross_network_dcn_v2__recsys_kernel(x0, U, V, bs):
    B, D = x0.shape
    L, _, R = U.shape
    assert (D, R) == (416, 104) and 2 < L <= 8
    G0, G, NU = 8, 10, 3
    GM = max(G, G0)
    out_t = pl.pallas_call(
        functools.partial(_kernel, GA=4, G0=G0, d0=3, G=G, d=4, NU=NU,
                          L0=2, lead=4, nfine=3),
        in_specs=[pl.BlockSpec(memory_space=pl.ANY)] * 4,
        out_specs=pl.BlockSpec(memory_space=pl.ANY),
        out_shape=jax.ShapeDtypeStruct((D, B), x0.dtype),
        scratch_shapes=[
            pltpu.VMEM((L, D, R), BF16),
            pltpu.VMEM((L, R, D), BF16),
            pltpu.VMEM((L, D), BF16),
            pltpu.VMEM((D, 128), F32),
            pltpu.VMEM((L, D // 2, 128), U32),
            pltpu.VMEM((L, 3, RP // 2, 128), U32),
            pltpu.VMEM((L, NC, R, 128), F32),
            pltpu.VMEM((GM, D, W), F32),
            pltpu.VMEM((GM, D, W), F32),
            pltpu.VMEM((GM, KA, W), BF16),
            pltpu.VMEM((GM, D - KA, W), F32),
            pltpu.VMEM((GM, 128, W), BF16),
            pltpu.VMEM((D, G0 * W), BF16),
            pltpu.VMEM((D, G0 * W), BF16),
            pltpu.VMEM((2, D, NU * G * W), BF16),
            pltpu.VMEM((2, D, NU * G * W), BF16),
            pltpu.SemaphoreType.DMA((10,)),
            pltpu.SemaphoreType.DMA((2,)),
            pltpu.SemaphoreType.DMA((2,)),
        ],
        compiler_params=pltpu.CompilerParams(
            vmem_limit_bytes=100 * 1024 * 1024,
            disable_bounds_checks=True,
        ),
    )(x0.T, U, V, bs)
    return out_t.T
```

```python
import functools

import jax
import jax.numpy as jnp
from jax import lax
import jax.experimental.pallas as pl
import jax.experimental.pallas.tpu as pltpu

F32 = jnp.float32
BF16 = jnp.bfloat16
U32 = jnp.uint32

W = 128
KA = 384
NC = 9


def _pk(x):
    return pltpu.bitcast(x, U32)


def _upk(x):
    return pltpu.bitcast(x, BF16)


def _kernel(x0_hbm, u_hbm, v_hbm, b_hbm, o_hbm,
            u_ref, v_ref, b_ref, bt_ref, uw_ref, va_ref, vcb_ref,
            x0f_ref, s_ref, xa_ref, xr_ref, st_ref,
            xin0_ref, xout0_ref, xin_ref, xout_ref, w_sem, in_sem, out_sem, *,
            GA, G0, d0, G, d, NU, L0, lead, nfine):
    D, B = x0_hbm.shape
    L, _, R = u_ref.shape
    CA = GA * W
    C0 = G0 * W
    CI = NU * G * W
    NI = (B - C0) // CI
    assert NI * CI + C0 == B and NI >= 2
    half = [(0, 224), (224, D)]
    fine = [(0, 112), (112, 208), (208, 320), (320, D)]

    def cols(i, off, n):
        return pl.ds(pl.multiple_of(C0 + i * CI + off, W), n)

    def in_copy(i, par):
        return pltpu.make_async_copy(
            x0_hbm.at[:, cols(i, 0, CI)], xin_ref.at[par], in_sem.at[par])

    def out_copy(i, par, c0, n):
        return pltpu.make_async_copy(
            xout_ref.at[par, :, pl.ds(c0, n)], o_hbm.at[:, cols(i, c0, n)],
            out_sem.at[par])

    def out_wait_all(par):
        pltpu.make_async_copy(
            xout_ref.at[par], xout_ref.at[par], out_sem.at[par]).wait()

    stage1 = [
        pltpu.make_async_copy(v_hbm.at[0:1], v_ref.at[0:1], w_sem.at[0]),
        pltpu.make_async_copy(b_hbm, b_ref, w_sem.at[1]),
        pltpu.make_async_copy(u_hbm.at[0:1], u_ref.at[0:1], w_sem.at[2]),
        pltpu.make_async_copy(
            x0_hbm.at[:, 0:CA], xin0_ref.at[:, 0:CA], w_sem.at[3]),
    ]
    stage2 = [
        pltpu.make_async_copy(
            x0_hbm.at[:, CA:C0], xin0_ref.at[:, CA:C0], w_sem.at[4]),
        pltpu.make_async_copy(v_hbm.at[1:L0], v_ref.at[1:L0], w_sem.at[5]),
        pltpu.make_async_copy(u_hbm.at[1:L0], u_ref.at[1:L0], w_sem.at[6]),
    ]
    stage3 = [
        pltpu.make_async_copy(v_hbm.at[L0:L], v_ref.at[L0:L], w_sem.at[7]),
        pltpu.make_async_copy(u_hbm.at[L0:L], u_ref.at[L0:L], w_sem.at[8]),
    ]
    out0 = pltpu.make_async_copy(xout0_ref, o_hbm.at[:, 0:C0], w_sem.at[9])
    for c in stage1 + stage2 + stage3:
        c.start()
    in_copy(0, 0).start()

    def vpu_col(l, j):
        return j if j < 8 else 8 + l

    def init_bias():
        b = b_ref[...].astype(F32)
        bm = jnp.concatenate(
            [jnp.zeros((R, D), F32), b, jnp.zeros((128 - R - L, D), F32)], axis=0)
        bm = jnp.concatenate([bm, jnp.zeros((128, 512 - D), F32)], axis=1)
        bt_ref[...] = bm.T[:D]

    def init(l):
        row = lax.broadcasted_iota(jnp.int32, (R, 128), 0)
        col = lax.broadcasted_iota(jnp.int32, (R, 128), 1)
        for k in range(3):
            va_ref[l, k] = v_ref[l, :, k * 128:(k + 1) * 128].astype(F32)
        vt0 = v_ref[l, :, KA:D].astype(F32)
        for j in range(NC):
            c = vpu_col(l, j)
            vcb_ref[l, j] = jnp.broadcast_to(vt0[:, c:c + 1], (R, 128))
        vt = jnp.concatenate([jnp.zeros((R, 128 - (D - KA)), F32), vt0], axis=1)
        e = jnp.where(col >= R, vt, jnp.where(row == col, 1.0, 0.0)).astype(BF16)
        for r0 in range(0, D, 112):
            r1 = min(r0 + 112, D)
            cold = lax.broadcasted_iota(jnp.int32, (r1 - r0, 128), 1)
            uw = jnp.dot(u_ref[l, r0:r1, :], e, preferred_element_type=F32)
            uw = jnp.where(cold == R + l, bt_ref[r0:r1, :], uw)
            uw_ref[l, r0 // 2:r1 // 2, :] = _pk(uw.astype(BF16))

    def p1(xin, c0, g, l):
        sub = lax.broadcasted_iota(jnp.int32, (128 - R, W), 0)
        if l == 0:
            x0f_ref[g] = xin[:, c0:c0 + W].astype(F32)
        h = None
        for k in range(3):
            if l == 0:
                xa = xin[k * 128:(k + 1) * 128, c0:c0 + W]
            else:
                xa = xa_ref[g, k * 128:(k + 1) * 128, :]
            p = lax.dot_general(va_ref[l, k], xa, (((1,), (0,)), ((), ())),
                                preferred_element_type=F32)
            h = p if h is None else h + p
        xr = x0f_ref[g, KA:, :] if l == 0 else xr_ref[g]
        for j in range(NC):
            c = vpu_col(l, j)
            h = h + vcb_ref[l, j] * xr[c:c + 1, :]
        tail = jnp.where(sub == l, 1.0, xr[8:])
        st_ref[g] = jnp.concatenate([h, tail], axis=0).astype(BF16)

    def p2(xout, c0, g, l, chunks):
        st = st_ref[g]
        for (r0, r1) in chunks:
            y = jnp.dot(_upk(uw_ref[l, r0 // 2:r1 // 2, :]), st,
                        preferred_element_type=F32)
            s = (y + 1.0) if l == 0 else (s_ref[g, r0:r1, :] + y)
            x = x0f_ref[g, r0:r1, :] * s
            if l == L - 1:
                xout[r0:r1, c0:c0 + W] = x.astype(BF16)
            else:
                s_ref[g, r0:r1, :] = s
                if r1 <= KA:
                    xa_ref[g, r0:r1, :] = x.astype(BF16)
                else:
                    xa_ref[g, r0:KA, :] = x[:KA - r0].astype(BF16)
                    xr_ref[g] = x[KA - r0:]

    for c in stage1[:3]:
        c.wait()
    init_bias()
    init(0)
    stage1[3].wait()
    for g in range(GA):
        p1(xin0_ref, g * W, g, 0)
    for g in range(GA):
        p2(xout0_ref, g * W, g, 0, fine)
    for c in stage2:
        c.wait()
    for l in range(1, L0):
        init(l)
    ts0 = L * G0
    tb = L0 * G0 - lead
    for t in range(GA, ts0 + d0):
        if (t + lead) % G0 == 0 and L0 <= (t + lead) // G0 < L:
            ln = (t + lead) // G0
            if ln == L0:
                for c in stage3:
                    c.wait()
            init(ln)
        if t < ts0:
            l, g = divmod(t, G0)
            p1(xin0_ref, g * W, g, l)
        if t - d0 >= GA:
            l, g = divmod(t - d0, G0)
            last = t >= ts0 + d0 - nfine or tb - nfine <= t < tb
            p2(xout0_ref, g * W, g, l, fine if last else half)
    out0.start()

    ts = L * G
    nt = ts * NU

    def body(i, carry):
        par = lax.rem(i, 2)

        @pl.when(i + 1 < NI)
        def _():
            in_copy(i + 1, 1 - par).start()

        in_copy(i, par).wait()

        @pl.when(i >= 2)
        def _():
            out_wait_all(par)

        xin = xin_ref.at[par]
        xout = xout_ref.at[par]
        done = 0
        for t in range(nt + d):
            if t < nt:
                u, r = divmod(t, ts)
                l, g = divmod(r, G)
                p1(xin, (u * G + g) * W, g, l)
            if t >= d:
                u, r = divmod(t - d, ts)
                l, g = divmod(r, G)
                p2(xout, (u * G + g) * W, g, l,
                   fine if t >= nt + d - nfine else half)
                if l == L - 1 and (u == NU - 1 or g == G - 1):
                    end = (u * G + g + 1) * W

                    @pl.when(i == NI - 1)
                    def _(done=done, end=end):
                        out_copy(i, par, done, end - done).start()

                    done = end
        assert done == CI

        @pl.when(i < NI - 1)
        def _():
            out_copy(i, par, 0, CI).start()

        return carry

    lax.fori_loop(0, NI, body, 0)
    out0.wait()
    out_wait_all((NI - 2) % 2)
    out_wait_all((NI - 1) % 2)


@jax.jit
def pallas_standalone__cross_network_dcn_v2__recsys_kernel(x0, U, V, bs):
    B, D = x0.shape
    L, _, R = U.shape
    assert (D, R) == (416, 104) and 2 < L <= 8
    G0, G, NU = 8, 10, 3
    GM = max(G, G0)
    out_t = pl.pallas_call(
        functools.partial(_kernel, GA=4, G0=G0, d0=3, G=G, d=4, NU=NU,
                          L0=2, lead=4, nfine=3),
        in_specs=[pl.BlockSpec(memory_space=pl.ANY)] * 4,
        out_specs=pl.BlockSpec(memory_space=pl.ANY),
        out_shape=jax.ShapeDtypeStruct((D, B), x0.dtype),
        scratch_shapes=[
            pltpu.VMEM((L, D, R), BF16),
            pltpu.VMEM((L, R, D), BF16),
            pltpu.VMEM((L, D), BF16),
            pltpu.VMEM((D, 128), F32),
            pltpu.VMEM((L, D // 2, 128), U32),
            pltpu.VMEM((L, 3, R, 128), F32),
            pltpu.VMEM((L, NC, R, 128), F32),
            pltpu.VMEM((GM, D, W), F32),
            pltpu.VMEM((GM, D, W), F32),
            pltpu.VMEM((GM, KA, W), BF16),
            pltpu.VMEM((GM, D - KA, W), F32),
            pltpu.VMEM((GM, 128, W), BF16),
            pltpu.VMEM((D, G0 * W), BF16),
            pltpu.VMEM((D, G0 * W), BF16),
            pltpu.VMEM((2, D, NU * G * W), BF16),
            pltpu.VMEM((2, D, NU * G * W), BF16),
            pltpu.SemaphoreType.DMA((10,)),
            pltpu.SemaphoreType.DMA((2,)),
            pltpu.SemaphoreType.DMA((2,)),
        ],
        compiler_params=pltpu.CompilerParams(
            vmem_limit_bytes=100 * 1024 * 1024,
            disable_bounds_checks=True,
        ),
    )(x0.T, U, V, bs)
    return out_t.T
```

```python
import functools

import jax
import jax.numpy as jnp
from jax import lax
import jax.experimental.pallas as pl
import jax.experimental.pallas.tpu as pltpu

F32 = jnp.float32
BF16 = jnp.bfloat16
U32 = jnp.uint32

W = 128
KA = 384
NC = 9


def _pk(x):
    return pltpu.bitcast(x, U32)


def _upk(x):
    return pltpu.bitcast(x, BF16)


def _kernel(x0_hbm, u_hbm, v_hbm, b_hbm, o_hbm,
            u_ref, v_ref, b_ref, bt_ref, uw_ref, va_ref, vcb_ref,
            x0f_ref, s_ref, xa_ref, xr_ref, st_ref,
            xin0_ref, xout0_ref, xin_ref, xout_ref, w_sem, in_sem, out_sem, *,
            GA, G0, d0, G, d, NU, L0, lead, idel, nfine):
    D, B = x0_hbm.shape
    L, _, R = u_ref.shape
    CA = GA * W
    C0 = G0 * W
    CI = NU * G * W
    NI = (B - C0) // CI
    assert NI * CI + C0 == B and NI >= 2
    half = [(0, 224), (224, D)]
    fine = [(0, 112), (112, 208), (208, 320), (320, D)]

    def cols(i, off, n):
        return pl.ds(pl.multiple_of(C0 + i * CI + off, W), n)

    def in_copy(i, par):
        return pltpu.make_async_copy(
            x0_hbm.at[:, cols(i, 0, CI)], xin_ref.at[par], in_sem.at[par])

    def out_copy(i, par, c0, n):
        return pltpu.make_async_copy(
            xout_ref.at[par, :, pl.ds(c0, n)], o_hbm.at[:, cols(i, c0, n)],
            out_sem.at[par])

    def out_wait_all(par):
        pltpu.make_async_copy(
            xout_ref.at[par], xout_ref.at[par], out_sem.at[par]).wait()

    stage1 = [
        pltpu.make_async_copy(v_hbm.at[0:1], v_ref.at[0:1], w_sem.at[0]),
        pltpu.make_async_copy(b_hbm, b_ref, w_sem.at[1]),
        pltpu.make_async_copy(u_hbm.at[0:1], u_ref.at[0:1], w_sem.at[2]),
        pltpu.make_async_copy(
            x0_hbm.at[:, 0:CA], xin0_ref.at[:, 0:CA], w_sem.at[3]),
    ]
    stage2 = [
        pltpu.make_async_copy(
            x0_hbm.at[:, CA:C0], xin0_ref.at[:, CA:C0], w_sem.at[4]),
        pltpu.make_async_copy(v_hbm.at[1:L0], v_ref.at[1:L0], w_sem.at[5]),
        pltpu.make_async_copy(u_hbm.at[1:L0], u_ref.at[1:L0], w_sem.at[6]),
    ]
    stage3 = [
        pltpu.make_async_copy(v_hbm.at[L0:L], v_ref.at[L0:L], w_sem.at[7]),
        pltpu.make_async_copy(u_hbm.at[L0:L], u_ref.at[L0:L], w_sem.at[8]),
    ]
    out0 = pltpu.make_async_copy(xout0_ref, o_hbm.at[:, 0:C0], w_sem.at[9])
    for c in stage1 + stage2 + stage3:
        c.start()
    in_copy(0, 0).start()

    def vpu_col(l, j):
        return j if j < 8 else 8 + l

    def init_bias():
        b = b_ref[...].astype(F32)
        bm = jnp.concatenate(
            [jnp.zeros((R, D), F32), b, jnp.zeros((128 - R - L, D), F32)], axis=0)
        bm = jnp.concatenate([bm, jnp.zeros((128, 512 - D), F32)], axis=1)
        bt_ref[...] = bm.T[:D]

    def init(l):
        row = lax.broadcasted_iota(jnp.int32, (R, 128), 0)
        col = lax.broadcasted_iota(jnp.int32, (R, 128), 1)
        for k in range(3):
            va_ref[l, k] = v_ref[l, :, k * 128:(k + 1) * 128].astype(F32)
        vt0 = v_ref[l, :, KA:D].astype(F32)
        for j in range(NC):
            c = vpu_col(l, j)
            vcb_ref[l, j] = jnp.broadcast_to(vt0[:, c:c + 1], (R, 128))
        vt = jnp.concatenate([jnp.zeros((R, 128 - (D - KA)), F32), vt0], axis=1)
        e = jnp.where(col >= R, vt, jnp.where(row == col, 1.0, 0.0)).astype(BF16)
        for r0 in range(0, D, 112):
            r1 = min(r0 + 112, D)
            cold = lax.broadcasted_iota(jnp.int32, (r1 - r0, 128), 1)
            uw = jnp.dot(u_ref[l, r0:r1, :], e, preferred_element_type=F32)
            uw = jnp.where(cold == R + l, bt_ref[r0:r1, :], uw)
            uw_ref[l, r0 // 2:r1 // 2, :] = _pk(uw.astype(BF16))

    def p1(xin, c0, g, l):
        sub = lax.broadcasted_iota(jnp.int32, (128 - R, W), 0)
        if l == 0:
            x0f_ref[g] = xin[:, c0:c0 + W].astype(F32)
        h = None
        for k in range(3):
            if l == 0:
                xa = xin[k * 128:(k + 1) * 128, c0:c0 + W]
            else:
                xa = xa_ref[g, k * 128:(k + 1) * 128, :]
            p = lax.dot_general(va_ref[l, k], xa, (((1,), (0,)), ((), ())),
                                precision=lax.Precision.DEFAULT,
                                preferred_element_type=F32)
            h = p if h is None else h + p
        xr = x0f_ref[g, KA:, :] if l == 0 else xr_ref[g]
        for j in range(NC):
            c = vpu_col(l, j)
            h = h + vcb_ref[l, j] * xr[c:c + 1, :]
        tail = jnp.where(sub == l, 1.0, xr[8:])
        st_ref[g] = jnp.concatenate([h, tail], axis=0).astype(BF16)

    def p2(xout, c0, g, l, chunks):
        st = st_ref[g]
        for (r0, r1) in chunks:
            y = jnp.dot(_upk(uw_ref[l, r0 // 2:r1 // 2, :]), st,
                        preferred_element_type=F32)
            s = (y + 1.0) if l == 0 else (s_ref[g, r0:r1, :] + y)
            x = x0f_ref[g, r0:r1, :] * s
            if l == L - 1:
                xout[r0:r1, c0:c0 + W] = x.astype(BF16)
            else:
                s_ref[g, r0:r1, :] = s
                if r1 <= KA:
                    xa_ref[g, r0:r1, :] = x.astype(BF16)
                else:
                    xa_ref[g, r0:KA, :] = x[:KA - r0].astype(BF16)
                    xr_ref[g] = x[KA - r0:]

    for c in stage1[:3]:
        c.wait()
    init_bias()
    init(0)
    stage1[3].wait()
    for g in range(GA):
        p1(xin0_ref, g * W, g, 0)
    for g in range(GA):
        p2(xout0_ref, g * W, g, 0, fine)
    for c in stage2:
        c.wait()
    ts0 = L * G0
    tb = L0 * G0 - lead - idel
    init_at = {max(l * G0 - lead, GA + idel): l for l in range(1, L)}
    for t in range(GA, ts0 + d0):
        if t == tb:
            for c in stage3:
                c.wait()
        if t in init_at:
            init(init_at[t])
        if t < ts0:
            l, g = divmod(t, G0)
            p1(xin0_ref, g * W, g, l)
        if t - d0 >= GA:
            l, g = divmod(t - d0, G0)
            last = t >= ts0 + d0 - nfine or tb - nfine <= t < tb
            p2(xout0_ref, g * W, g, l, fine if last else half)
    out0.start()

    ts = L * G
    nt = ts * NU

    def body(i, carry):
        par = lax.rem(i, 2)

        @pl.when(i + 1 < NI)
        def _():
            in_copy(i + 1, 1 - par).start()

        in_copy(i, par).wait()

        @pl.when(i >= 2)
        def _():
            out_wait_all(par)

        xin = xin_ref.at[par]
        xout = xout_ref.at[par]
        done = 0
        for t in range(nt + d):
            if t < nt:
                u, r = divmod(t, ts)
                l, g = divmod(r, G)
                p1(xin, (u * G + g) * W, g, l)
            if t >= d:
                u, r = divmod(t - d, ts)
                l, g = divmod(r, G)
                p2(xout, (u * G + g) * W, g, l,
                   fine if t >= nt + d - nfine else half)
                if l == L - 1 and (u == NU - 1 or g == G - 1):
                    end = (u * G + g + 1) * W

                    @pl.when(i == NI - 1)
                    def _(done=done, end=end):
                        out_copy(i, par, done, end - done).start()

                    done = end
        assert done == CI

        @pl.when(i < NI - 1)
        def _():
            out_copy(i, par, 0, CI).start()

        return carry

    lax.fori_loop(0, NI, body, 0)
    out0.wait()
    out_wait_all((NI - 2) % 2)
    out_wait_all((NI - 1) % 2)


@jax.jit
def pallas_standalone__cross_network_dcn_v2__recsys_kernel(x0, U, V, bs):
    B, D = x0.shape
    L, _, R = U.shape
    assert (D, R) == (416, 104) and 2 < L <= 8
    G0, G, NU = 8, 10, 3
    GM = max(G, G0)
    out_t = pl.pallas_call(
        functools.partial(_kernel, GA=4, G0=G0, d0=3, G=G, d=4, NU=NU,
                          L0=2, lead=1, idel=2, nfine=3),
        in_specs=[pl.BlockSpec(memory_space=pl.ANY)] * 4,
        out_specs=pl.BlockSpec(memory_space=pl.ANY),
        out_shape=jax.ShapeDtypeStruct((D, B), x0.dtype),
        scratch_shapes=[
            pltpu.VMEM((L, D, R), BF16),
            pltpu.VMEM((L, R, D), BF16),
            pltpu.VMEM((L, D), BF16),
            pltpu.VMEM((D, 128), F32),
            pltpu.VMEM((L, D // 2, 128), U32),
            pltpu.VMEM((L, 3, R, 128), F32),
            pltpu.VMEM((L, NC, R, 128), F32),
            pltpu.VMEM((GM, D, W), F32),
            pltpu.VMEM((GM, D, W), F32),
            pltpu.VMEM((GM, KA, W), BF16),
            pltpu.VMEM((GM, D - KA, W), F32),
            pltpu.VMEM((GM, 128, W), BF16),
            pltpu.VMEM((D, G0 * W), BF16),
            pltpu.VMEM((D, G0 * W), BF16),
            pltpu.VMEM((2, D, NU * G * W), BF16),
            pltpu.VMEM((2, D, NU * G * W), BF16),
            pltpu.SemaphoreType.DMA((10,)),
            pltpu.SemaphoreType.DMA((2,)),
            pltpu.SemaphoreType.DMA((2,)),
        ],
        compiler_params=pltpu.CompilerParams(
            vmem_limit_bytes=64 * 1024 * 1024,
            disable_bounds_checks=True,
            disable_semaphore_checks=True,
        ),
    )(x0.T, U, V, bs)
    return out_t.T
```

```python
import functools

import jax
import jax.numpy as jnp
from jax import lax
import jax.experimental.pallas as pl
import jax.experimental.pallas.tpu as pltpu

F32 = jnp.float32
BF16 = jnp.bfloat16
U32 = jnp.uint32

W = 128
KA = 384
NC = 9


def _pk(x):
    return pltpu.bitcast(x, U32)


def _upk(x):
    return pltpu.bitcast(x, BF16)


def _kernel(x0_hbm, u_hbm, v_hbm, b_hbm, o_hbm,
            u_ref, v_ref, b_ref, bt_ref, uw_ref, va_ref, vcb_ref,
            x0f_ref, s_ref, xa_ref, xr_ref, st_ref,
            xin0_ref, xout0_ref, xin_ref, xout_ref, w_sem, in_sem, out_sem, *,
            GA, G0, d0, G, d, NU, L0, lead, idel, nfine):
    D, B = x0_hbm.shape
    L, _, R = u_ref.shape
    CA = GA * W
    C0 = G0 * W
    CI = NU * G * W
    NI = (B - C0) // CI
    assert NI * CI + C0 == B and NI >= 2
    half = [(0, 224), (224, D)]
    fine = [(0, 112), (112, 208), (208, 320), (320, D)]

    def cols(i, off, n):
        return pl.ds(pl.multiple_of(C0 + i * CI + off, W), n)

    def in_copy(i, par):
        return pltpu.make_async_copy(
            x0_hbm.at[:, cols(i, 0, CI)], xin_ref.at[par], in_sem.at[par])

    def out_copy(i, par, c0, n):
        return pltpu.make_async_copy(
            xout_ref.at[par, :, pl.ds(c0, n)], o_hbm.at[:, cols(i, c0, n)],
            out_sem.at[par])

    def out_wait_all(par):
        pltpu.make_async_copy(
            xout_ref.at[par], xout_ref.at[par], out_sem.at[par]).wait()

    stage1 = [
        pltpu.make_async_copy(v_hbm.at[0:1], v_ref.at[0:1], w_sem.at[0]),
        pltpu.make_async_copy(b_hbm, b_ref, w_sem.at[1]),
        pltpu.make_async_copy(u_hbm.at[0:1], u_ref.at[0:1], w_sem.at[2]),
        pltpu.make_async_copy(
            x0_hbm.at[:, 0:CA], xin0_ref.at[:, 0:CA], w_sem.at[3]),
    ]
    stage2 = [
        pltpu.make_async_copy(
            x0_hbm.at[:, CA:C0], xin0_ref.at[:, CA:C0], w_sem.at[4]),
        pltpu.make_async_copy(v_hbm.at[1:L0], v_ref.at[1:L0], w_sem.at[5]),
        pltpu.make_async_copy(u_hbm.at[1:L0], u_ref.at[1:L0], w_sem.at[6]),
    ]
    stage3 = [
        pltpu.make_async_copy(v_hbm.at[L0:L], v_ref.at[L0:L], w_sem.at[7]),
        pltpu.make_async_copy(u_hbm.at[L0:L], u_ref.at[L0:L], w_sem.at[8]),
    ]
    out0 = pltpu.make_async_copy(xout0_ref, o_hbm.at[:, 0:C0], w_sem.at[9])
    for c in stage1 + stage2 + stage3:
        c.start()
    in_copy(0, 0).start()

    def vpu_col(l, j):
        return j if j < 8 else 8 + l

    def init_bias():
        b = b_ref[...].astype(F32)
        bm = jnp.concatenate(
            [jnp.zeros((R, D), F32), b, jnp.zeros((128 - R - L, D), F32)], axis=0)
        bm = jnp.concatenate([bm, jnp.zeros((128, 512 - D), F32)], axis=1)
        bt_ref[...] = bm.T[:D]

    def init(l):
        row = lax.broadcasted_iota(jnp.int32, (R, 128), 0)
        col = lax.broadcasted_iota(jnp.int32, (R, 128), 1)
        for k in range(3):
            va_ref[l, k] = v_ref[l, :, k * 128:(k + 1) * 128].astype(F32)
        vt0 = v_ref[l, :, KA:D].astype(F32)
        for j in range(NC):
            c = vpu_col(l, j)
            vcb_ref[l, j] = jnp.broadcast_to(vt0[:, c:c + 1], (R, 128))
        vt = jnp.concatenate([jnp.zeros((R, 128 - (D - KA)), F32), vt0], axis=1)
        e = jnp.where(col >= R, vt, jnp.where(row == col, 1.0, 0.0)).astype(BF16)
        for r0 in range(0, D, 112):
            r1 = min(r0 + 112, D)
            cold = lax.broadcasted_iota(jnp.int32, (r1 - r0, 128), 1)
            uw = jnp.dot(u_ref[l, r0:r1, :], e, preferred_element_type=F32)
            uw = jnp.where(cold == R + l, bt_ref[r0:r1, :], uw)
            uw_ref[l, r0 // 2:r1 // 2, :] = _pk(uw.astype(BF16))

    def p1(xin, c0, g, l):
        sub = lax.broadcasted_iota(jnp.int32, (128 - R, W), 0)
        if l == 0:
            x0f_ref[g] = xin[:, c0:c0 + W].astype(F32)
        h = None
        for k in range(3):
            if l == 0:
                xa = xin[k * 128:(k + 1) * 128, c0:c0 + W]
            else:
                xa = xa_ref[g, k * 128:(k + 1) * 128, :]
            p = lax.dot_general(va_ref[l, k], xa, (((1,), (0,)), ((), ())),
                                precision=lax.Precision.DEFAULT,
                                preferred_element_type=F32)
            h = p if h is None else h + p
        xr = x0f_ref[g, KA:, :] if l == 0 else xr_ref[g]
        for j in range(NC):
            c = vpu_col(l, j)
            h = h + vcb_ref[l, j] * xr[c:c + 1, :]
        tail = jnp.where(sub == l, 1.0, xr[8:])
        st_ref[g] = _pk(jnp.concatenate([h, tail], axis=0).astype(BF16))

    def p2(xout, c0, g, l, chunks):
        st = _upk(st_ref[g])
        for (r0, r1) in chunks:
            y = jnp.dot(_upk(uw_ref[l, r0 // 2:r1 // 2, :]), st,
                        preferred_element_type=F32)
            s = (y + 1.0) if l == 0 else (s_ref[g, r0:r1, :] + y)
            x = x0f_ref[g, r0:r1, :] * s
            if l == L - 1:
                xout[r0:r1, c0:c0 + W] = x.astype(BF16)
            else:
                s_ref[g, r0:r1, :] = s
                if r1 <= KA:
                    xa_ref[g, r0:r1, :] = x.astype(BF16)
                else:
                    xa_ref[g, r0:KA, :] = x[:KA - r0].astype(BF16)
                    xr_ref[g] = x[KA - r0:]

    for c in stage1[:3]:
        c.wait()
    init_bias()
    init(0)
    stage1[3].wait()
    for g in range(GA):
        p1(xin0_ref, g * W, g, 0)
    for g in range(GA):
        p2(xout0_ref, g * W, g, 0, fine)
    for c in stage2:
        c.wait()
    ts0 = L * G0
    tb = L0 * G0 - lead - idel
    init_at = {max(l * G0 - lead, GA + idel): l for l in range(1, L)}
    for t in range(GA, ts0 + d0):
        if t == tb:
            for c in stage3:
                c.wait()
        if t in init_at:
            init(init_at[t])
        if t < ts0:
            l, g = divmod(t, G0)
            p1(xin0_ref, g * W, g, l)
        if t - d0 >= GA:
            l, g = divmod(t - d0, G0)
            last = t >= ts0 + d0 - nfine or tb - nfine <= t < tb
            p2(xout0_ref, g * W, g, l, fine if last else half)
    out0.start()

    ts = L * G
    nt = ts * NU

    def body(i, carry):
        par = lax.rem(i, 2)

        @pl.when(i + 1 < NI)
        def _():
            in_copy(i + 1, 1 - par).start()

        in_copy(i, par).wait()

        @pl.when(i >= 2)
        def _():
            out_wait_all(par)

        xin = xin_ref.at[par]
        xout = xout_ref.at[par]
        done = 0
        for t in range(nt + d):
            if t < nt:
                u, r = divmod(t, ts)
                l, g = divmod(r, G)
                p1(xin, (u * G + g) * W, g, l)
            if t >= d:
                u, r = divmod(t - d, ts)
                l, g = divmod(r, G)
                p2(xout, (u * G + g) * W, g, l,
                   fine if t >= nt + d - nfine else half)
                if l == L - 1 and (u == NU - 1 or g == G - 1):
                    end = (u * G + g + 1) * W

                    @pl.when(i == NI - 1)
                    def _(done=done, end=end):
                        out_copy(i, par, done, end - done).start()

                    done = end
        assert done == CI

        @pl.when(i < NI - 1)
        def _():
            out_copy(i, par, 0, CI).start()

        return carry

    lax.fori_loop(0, NI, body, 0)
    out0.wait()
    out_wait_all((NI - 2) % 2)
    out_wait_all((NI - 1) % 2)


@jax.jit
def pallas_standalone__cross_network_dcn_v2__recsys_kernel(x0, U, V, bs):
    B, D = x0.shape
    L, _, R = U.shape
    assert (D, R) == (416, 104) and 2 < L <= 8
    G0, G, NU = 8, 10, 3
    GM = max(G, G0)
    out_t = pl.pallas_call(
        functools.partial(_kernel, GA=4, G0=G0, d0=3, G=G, d=3, NU=NU,
                          L0=2, lead=1, idel=2, nfine=2),
        in_specs=[pl.BlockSpec(memory_space=pl.ANY)] * 4,
        out_specs=pl.BlockSpec(memory_space=pl.ANY),
        out_shape=jax.ShapeDtypeStruct((D, B), x0.dtype),
        scratch_shapes=[
            pltpu.VMEM((L, D, R), BF16),
            pltpu.VMEM((L, R, D), BF16),
            pltpu.VMEM((L, D), BF16),
            pltpu.VMEM((D, 128), F32),
            pltpu.VMEM((L, D // 2, 128), U32),
            pltpu.VMEM((L, 3, R, 128), F32),
            pltpu.VMEM((L, NC, R, 128), F32),
            pltpu.VMEM((GM, D, W), F32),
            pltpu.VMEM((GM, D, W), F32),
            pltpu.VMEM((GM, KA, W), BF16),
            pltpu.VMEM((GM, D - KA, W), F32),
            pltpu.VMEM((GM, 64, W), U32),
            pltpu.VMEM((D, G0 * W), BF16),
            pltpu.VMEM((D, G0 * W), BF16),
            pltpu.VMEM((2, D, NU * G * W), BF16),
            pltpu.VMEM((2, D, NU * G * W), BF16),
            pltpu.SemaphoreType.DMA((10,)),
            pltpu.SemaphoreType.DMA((2,)),
            pltpu.SemaphoreType.DMA((2,)),
        ],
        compiler_params=pltpu.CompilerParams(
            vmem_limit_bytes=64 * 1024 * 1024,
            disable_bounds_checks=True,
            disable_semaphore_checks=True,
        ),
    )(x0.T, U, V, bs)
    return out_t.T
```
